```python
import os as _os
_os.environ.setdefault('JAX_PLATFORMS', 'cpu')
import jax
import jax.numpy as jnp

def _softmax(x, axis=-1):
    return jax.nn.softmax(x, axis=axis)

def _gelu(x):
    return jax.nn.gelu(x, approximate=True)

def _silu(x):
    return jax.nn.silu(x)

def _sigmoid(x):
    return jax.nn.sigmoid(x)

def _layernorm(x, axis=-1, eps=1e-05):
    m = jnp.mean(x, axis=axis, keepdims=True)
    v = jnp.var(x, axis=axis, keepdims=True)
    return (x - m) / jnp.sqrt(v + eps)

def _scatter_add(tgt, idx, src, axis=0):
    return tgt.at[idx].add(src)

def _segment_sum(src, seg, n):
    return jax.ops.segment_sum(src, seg, n)

class _Rng:

    def __init__(self, key):
        self._k = key

    def _next(self):
        self._k, sub = jax.random.split(self._k)
        return sub

    def normal(self, shape):
        return jax.random.normal(self._next(), shape, dtype=jnp.bfloat16)

    def randint(self, lo, hi, shape):
        return jax.random.randint(self._next(), shape, lo, hi, dtype=jnp.int32)

    def uniform(self, shape, lo=0.0, hi=1.0):
        return jax.random.uniform(self._next(), shape, jnp.bfloat16, lo, hi)

    def permutation(self, n):
        return jax.random.permutation(self._next(), n)
kernel_name = 'adaLN_cond__sliding_local_dilated__mixer_channel_mlp__prompt'

def setup_inputs():
    _rng = _Rng(jax.random.key(int.from_bytes(__import__("os").urandom(4), "little")))
    _w = lambda a: (lambda t: t.astype(jnp.bfloat16) if jnp.issubdtype(t.dtype, jnp.floating) else t)(jnp.asarray(a))

    def _A_setup():
        B, S, D = (1, 2048, 512)
        return {'x': _w((lambda *s: _rng.normal(s) * 0.05)(B, S, D)), 'wqkv': _w((lambda *s: _rng.normal(s) * 0.05)(D, 3 * D)), 'wo': _w((lambda *s: _rng.normal(s) * 0.05)(D, D))}
    _A_in = _A_setup()

    def _B_setup():
        B, S, D, F = (1, 2048, 512, 1792)
        return {'x': _w((lambda *s: _rng.normal(s) * 0.05)(B, S, D)), 'w1': _w((lambda *s: _rng.normal(s) * 0.8)(D, F) * D ** (-0.5)), 'b1': _w((lambda *s: _rng.normal(s) * 0.8)(F)), 'w2': _w((lambda *s: _rng.normal(s) * 0.8)(F, D) * F ** (-0.5)), 'b2': _w((lambda *s: _rng.normal(s) * 0.4)(D))}
    _B_in = _B_setup()
    return {'A_x': _A_in['x'], 'A_wqkv': _A_in['wqkv'], 'A_wo': _A_in['wo'], 'B_x': _B_in['x'], 'B_w1': _B_in['w1'], 'B_b1': _B_in['b1'], 'B_w2': _B_in['w2'], 'B_b2': _B_in['b2'], 'c': _w((lambda *s: _rng.normal(s) * 0.05)(1, 512) * 8.0), 'w_mod': _w((lambda *s: _rng.normal(s) * 0.05)(512, 6 * 512) * 512 ** (-0.5) * 8.0)}

def reference(A_x, A_wqkv, A_wo, B_x, B_w1, B_b1, B_w2, B_b2, c, w_mod):

    def _A_ref(x, wqkv, wo):
        B, S, D = x.shape
        H = 32
        Dh = D // H
        W, dil = (8, 2)
        qkv = (lambda x, *d: x.transpose(*d))((x @ wqkv).reshape(B, S, 3, H, Dh), 2, 0, 3, 1, 4)
        q, k, v = (qkv[0], qkv[1], qkv[2])
        scale = Dh ** (-0.5)
        pos = jnp.arange(S)
        off = jnp.arange(W) * dil
        idx = pos[:, None] - off[None, :]
        mask = idx >= 0
        idx_c = jnp.where(mask, idx, 0).reshape(-1)
        kg = k[:, :, idx_c, :].reshape(B, H, S, W, Dh)
        vg = v[:, :, idx_c, :].reshape(B, H, S, W, Dh)
        logits = jnp.einsum('bhsd,bhswd->bhsw', q, kg) * scale
        logits = jnp.where(mask[None, None, :, :], logits, -1000000000.0)
        attn = _softmax(logits, axis=-1)
        o = jnp.einsum('bhsw,bhswd->bhsd', attn, vg)
        return (lambda x, *d: x.transpose(*d))(o, 0, 2, 1, 3).reshape(B, S, D) @ wo

    def _B_ref(x, w1, b1, w2, b2):
        y = _layernorm(x, axis=-1)
        h = _gelu(jnp.einsum('bsd,df->bsf', y, w1) + b1)
        return jnp.einsum('bsf,fd->bsd', h, w2) + b2
    x = A_x
    mod = (_silu(c) @ w_mod).reshape(c.shape[0], 6, 1, -1)
    sa, ca, ga, sb, cb, gb = (mod[:, 0].copy(), mod[:, 1].copy(), mod[:, 2].copy(), mod[:, 3].copy(), mod[:, 4].copy(), mod[:, 5].copy())
    h = _layernorm(x, axis=-1) * (1 + ca) + sa
    x = x + ga * _A_ref(h, A_wqkv, A_wo)
    h = _layernorm(x, axis=-1) * (1 + cb) + sb
    x = x + gb * _B_ref(h, B_w1, B_b1, B_w2, B_b2)
    return x
```

```python
import functools
import heapq
import math

import jax
import jax.numpy as jnp
from jax import lax
from jax.experimental import pallas as pl
from jax.experimental.pallas import tpu as pltpu

S, D, F = 2048, 512, 1792
H, DH, W, DIL = 32, 16, 8, 2
EPS = 1e-5
LOG2E = math.log2(math.e)
GELU_A = (math.sqrt(2.0 / math.pi) * 0.044715) ** (1.0 / 3.0)
GELU_K = math.sqrt(2.0 / math.pi) / GELU_A
QK_A = math.sqrt(DH ** -0.5 * LOG2E)

TM = 256
NT, HM = S // TM, TM // 2
G = 32
NG = TM // G
NC = D // 128
HD, HF = D // 2, F // 2
Q = S // 4
HALO = 16
UP_COLS = (256, 256, 384)
PREP_ROWS = 16
f32, bf16, i32 = jnp.float32, jnp.bfloat16, jnp.int32

TUNING = dict(
    proj_after=(4, 6), one_hop=(1, 2), step=135, slack=930,
    due_attn=400, due_ln1=260, due_ln23=620, due_gelu=570, due_out=180, due_prep=30, due_w1=110, due_w2=130,
    end_attn=1300, end_ln1=1510, end_ln23=1610, end_gelu=960, end_prep=1440, qkv_to=40, w2_from=5, w2_to=-170,
    at_attn=0.76, at_ln23=0.75, len_ln23=1.2, len_out=20,
    lead_w=450, lead_w_more=150, lead_w_second=250, lead_mod=384,
)


def _pack(x):
    return pltpu.bitcast(x.astype(bf16), i32)


def _unpack(x):
    return pltpu.bitcast(x, bf16)


def _cat(xs, axis):
    xs = [x for x in xs if x.shape[axis]]
    return xs[0] if len(xs) == 1 else lax.concatenate(xs, axis)


def _fold(op, x, axis):
    while x.shape[axis] > 8:
        n = x.shape[axis] // 2
        x = op(lax.slice_in_dim(x, 0, n, axis=axis), lax.slice_in_dim(x, n, 2 * n, axis=axis))
    return x


def _lhs_ops(a11, a12, a21, a22):
    return [a11 + a22, a21 + a22, a11, a22, a11 + a12, a21 - a11, a12 - a22]


def _rhs_ops(b11, b12, b21, b22):
    return [b11 + b22, b11, b12 - b22, b21 - b11, b22, b11 + b12, b21 + b22]


def _top(m):
    return ((m[0] + m[3]) - m[4]) + m[6], m[2] + m[4]


def _bottom(m):
    return m[1] + m[3], ((m[0] - m[1]) + m[2]) + m[5]


def _rsqrt(v):
    return jnp.exp2(-0.5 * jnp.log2(v))


def _layer_norm(x, gain=1.0):
    mean = jnp.sum(x, axis=-1, keepdims=True)
    yield
    xc = x - mean * (1.0 / D)
    var = jnp.sum(xc * xc, axis=-1, keepdims=True)
    yield
    return xc * _rsqrt(var * (1.0 / (D * gain * gain)) + EPS / (gain * gain))


class _NotReady(Exception):
    pass


def _kernel(x_hbm, wqkv_hbm, wo_hbm, w1_hbm, b1_hbm, w2_hbm, b2_hbm, c_hbm, wmod_hbm, o_hbm,
            x_v, wqkv_v, wo_v, w1_v, w2_v, wmod_v, b1_v, b2_v, c_v, o_v,
            wp_s, wo_s, tq_s, t1_s, t2_s, sc_s, h0_s, h_s, a_s, y_s, g_s, q_s, k_s, v_s,
            in_sems, out_sems):
    cfg = TUNING

    copies = {}

    def fetch(name, src, dst):
        pltpu.make_async_copy(src, dst, in_sems.at[len(copies)]).start()
        copies[name] = (src, dst, len(copies))

    def fetch_x(t0, t1):
        fetch(("x", t0), x_hbm.at[0, t0 * TM:t1 * TM], x_v.at[t0 * TM:t1 * TM])

    def fetch_mod(n0, n1):
        fetch(("mod", n0), wmod_hbm.at[:, n0:n1], wmod_v.at[:, n0:n1])

    fetch("c", c_hbm, c_v)
    fetch_x(0, 1)
    for k in (0, HD):
        fetch_mod(k, k + HD)
        fetch_mod(D + k, D + k + HD)
        for n in range(0, 3 * D, D):
            fetch(("wqkv", k, n), wqkv_hbm.at[k:k + HD, n:n + D], wqkv_v.at[k:k + HD, n:n + D])
            if k == n == 0:
                fetch_x(1, 2)
    fetch_x(2, 3)
    fetch_x(3, 4)
    fetch("wo", wo_hbm, wo_v)
    fetch_x(4, NT)
    fetch_mod(2 * D, 3 * D)
    fetch_mod(3 * D, 5 * D)
    fetch("b1", b1_hbm, b1_v)
    fetch("b2", b2_hbm, b2_v)
    fetch("w1", w1_hbm, w1_v)
    fetch("w2", w2_hbm, w2_v)
    fetch_mod(5 * D, 6 * D)

    pltpu.make_async_copy(c_hbm, c_v, in_sems.at[0]).wait()
    cf = c_v[...].astype(f32)
    silu_c = cf * jax.nn.sigmoid(cf)
    start = jnp.broadcast_to(cf[:, 0:128], (8, 128))
    true = (pltpu.bitcast(start, i32) | 1) != 0

    masks = {}

    def spread(tile, shape):
        tile = _cat([_cat([tile] * (shape[-1] // 128), 1)] * (shape[-2] // 8), 0)
        return tile if len(shape) == 2 else lax.broadcast(tile, shape[:-2])

    def after(x, tok):
        if x.shape not in masks:
            masks[x.shape] = spread(true, x.shape)
        if tok.dtype != x.dtype:
            tok = pltpu.bitcast(tok, x.dtype)
        return lax.select(masks[x.shape], x, tok if tok.shape == x.shape else spread(tok, x.shape))

    def after_rows(x, r, toks):
        toks = [t if t.dtype == i32 else pltpu.bitcast(t, i32) for t in toks]
        while len(toks) > 2:
            toks = toks[2:] + [toks[0] ^ toks[1]]
        band = _cat([toks[n % len(toks)] for n in range(x.shape[1] // 128)], 1)
        return _cat([x[:r], after(x[r:r + 8], band), x[r + 8:]], 0)

    def arrived(name, tok):
        src, dst, k = copies[name]
        zero = after(jnp.zeros((8, 128), i32), tok)[0, 0]
        pltpu.make_async_copy(src, dst, in_sems.at[k + zero]).wait()

    written = {}

    def write(ref, r, n, val):
        ref[r:r + val.shape[0], n:n + val.shape[1]] = val
        written.setdefault(id(ref), set()).update(
            (r + i, n + j) for i in range(0, val.shape[0], 8) for j in range(0, val.shape[1], 128))

    def read(ref, r0, r1, n0, n1):
        have = written.get(id(ref), ())
        if any((r, n) not in have for r in range(r0, r1, 8) for n in range(n0, n1, 128)):
            raise _NotReady
        return ref[r0:r1, n0:n1]

    def write_lhs(ref, r, n, quad):
        done = []
        for i, op in enumerate(_lhs_ops(*quad)):
            row = i * Q + r // 4
            write(ref, row, n, _pack(op))
            if i >= 5:
                done += [ref[row:row + 8, m:m + 128] for m in range(n, n + op.shape[1], 128)]
        return done

    def write_group(ref, r, x):
        return write_lhs(ref, r, 0, (x[:16, :HD], x[:16, HD:], x[16:, :HD], x[16:, HD:]))

    vals = {}

    def interleave_heads(k, n0, tok):
        arrived(("wqkv", k, n0), tok)
        lane = lax.broadcasted_iota(i32, (HD // 2, 128), 1)
        quarter, head = (lane >> 2) & 3, lane & 31
        old = [pltpu.bitcast(wqkv_v[k:k + HD, n:n + 128], i32) for n in range(n0, n0 + D, 128)]
        for c in range(NC):
            z = old[(c - 3) % 4]
            for j in (2, 1, 0):
                z = jnp.where(quarter == j, old[(c - j) % 4], z)
            src = (head & 7) * DH + 4 * ((c - (head >> 3)) & 3) + (lane >> 5)
            write(wp_s, k // 2, n0 + c * 128, jnp.take_along_axis(z, src, axis=1))

    def right_operands(block, wait, ref, half_k, cols, half_n, n_out, rows, block_is_packed=False):
        def task(k0, n, tok):
            if wait and k0 == 0 and n == cols[0]:
                arrived(wait, tok)
            quad = [block(k, m) for k in (k0, half_k + k0) for m in (n, n + half_n)]
            done = []
            for i, op in enumerate(_rhs_ops(after(quad[0], tok), quad[1], quad[2], after(quad[3], tok))):
                if block_is_packed and i in (1, 4):
                    continue
                row, col = (i * half_k + k0) // 2, n_out + n - cols[0]
                write(ref, row, col, _pack(op))
                if i not in (1, 4):
                    done += [ref[row + j:row + j + 8, col:col + 128] for j in range(0, rows // 2, 8)]
            return done
        return [functools.partial(task, k0, n) for n in cols for k0 in range(0, half_k, rows)]

    def prepare_qkv(part):
        block = lambda k, n: _unpack(read(wp_s, k // 2, (k + PREP_ROWS) // 2, n, n + 128)).astype(f32)
        return right_operands(block, None, tq_s, HD, (part * D, part * D + 128), HD, part * HD, PREP_ROWS, True)

    def prepare_wo():
        def widen(n, tok):
            if n == 0:
                arrived("wo", tok)
            wo_s[n] = after(wo_v[:, n * 128:(n + 1) * 128].astype(f32), tok)

        def block(k, n):
            c, d = divmod(k // 32, 4)
            return _cat([wo_s[n // 128, pl.ds(128 * j + 4 * ((c - j) % 4) + d, 8, stride=DH), :]
                         for j in range(4)], 0)
        return ([functools.partial(widen, n) for n in range(NC)]
                + right_operands(block, None, tq_s, HD, (0, 128), HD, 3 * HD, 32))

    def prepare_w1():
        block = lambda k, n: w1_v[k:k + PREP_ROWS, n:n + 128].astype(f32)
        return right_operands(block, "w1", t1_s, HD, range(0, HF, 128), HF, 0, PREP_ROWS)

    def prepare_w2():
        block = lambda k, n: w2_v[k:k + PREP_ROWS, n:n + 128].astype(f32)
        return right_operands(block, "w2", t2_s, HF, (0, 128), HD, 0, PREP_ROWS)

    def biases(tok):
        arrived("b1", tok)
        vals["b1"] = b1_v[...].reshape(1, F).astype(f32) * GELU_A
        arrived("b2", tok)
        vals["b2"] = b2_v[...].reshape(1, D).astype(f32) * (2.0 * GELU_A)

    def shift_and_scale(k, tok):
        lhs = jnp.broadcast_to(silu_c.astype(bf16), (16, D))
        res = []
        for n in (k, D + k):
            arrived(("mod", n), tok)
            res.append(jnp.dot(lhs, wmod_v[:, n:n + HD], preferred_element_type=f32)[0:1])
        vals["sa", k], vals["ca", k] = res[0] * QK_A, (1.0 + res[1]) * QK_A
        if k:
            vals["sa"], vals["ca"] = [_cat([vals[name, 0], vals[name, k]], 1) for name in ("sa", "ca")]

    def column_of_c(tok):
        for n in range(0, D, 128):
            row = after(jnp.broadcast_to(silu_c[:, n:n + 128], (8, 128)), tok)[0:1]
            sc_s[n:n + 128, :] = jnp.broadcast_to(row, (128, 128)).T

    def modulation(index, name, post):
        parts, acc = [], {}

        def task(n, k, tok):
            if k == 0 and ("mod", n) in copies:
                arrived(("mod", n), tok)
            terms = wmod_v[k:k + 128, n:n + 128].astype(f32) * after(sc_s[k:k + 128, :], tok)
            acc[n] = _fold(jnp.add, terms, 0) + acc[n] if k else _fold(jnp.add, terms, 0)
            if k + 128 == D:
                parts.append(jnp.sum(acc[n], axis=0, keepdims=True))
                if len(parts) == NC:
                    vals[name] = post(_cat(parts, 1))
            return [acc[n]]
        return [functools.partial(task, n, k)
                for n in range(index * D, (index + 1) * D, 128) for k in range(0, D, 128)]

    def normalize(t, tok):
        arrived(("x", t), tok)
        x = x_v[t * TM:(t + 1) * TM, :].astype(f32)
        xc = x - jnp.sum(x, axis=-1, keepdims=True) * (1.0 / D)
        vals["xn", t] = xc * lax.rsqrt(jnp.sum(xc * xc, axis=-1, keepdims=True) * (1.0 / D) + EPS)

    def modulate(t, k, tok):
        h = vals["xn", t][:, k:k + HD] * vals["ca", k] + vals["sa", k]
        write(h0_s, t * HM, k, _pack(h))
        return h

    def first_norm(t):
        def task(r, tok):
            if r == t * TM and ("x", t) in copies:
                arrived(("x", t), tok)
            x = x_v[r:r + G, :].astype(f32)
            x = _cat([after(x[:, :128], tok), x[:, 128:]], 1)
            return write_group(h_s, r, (yield from _layer_norm(x)) * vals["ca"] + vals["sa"])
        return [functools.partial(task, r) for r in range(t * TM, (t + 1) * TM, G)]

    def put_qkv(part, c, r, blk):
        ref, r0 = (q_s, r) if part == 0 else ((k_s, v_s)[part - 1], HALO + r)
        ref[c, r0:r0 + blk.shape[0], :] = blk
        if part and r == 0:
            ref[c, 0:HALO, :] = jnp.broadcast_to(blk[0:1], (HALO, 128))
        written.setdefault("qkv", set()).update((part, c, r + i) for i in range(0, blk.shape[0], 8))

    def split_qkv(t, part):
        def task(j, tok):
            m = [p[16 * j:16 * j + 16] for p in vals["qkv", t, part]]
            for i, blk in enumerate(_top(m) + _bottom(m)):
                for c in range(2):
                    put_qkv(part, 2 * (i % 2) + c, t * TM + G * j + 16 * (i // 2), blk[:, c * 128:(c + 1) * 128])
        return [functools.partial(task, j) for j in range(NG)]

    def attention(t):
        pending = []

        def task(r, tok):
            assert all((p, c, r) in written["qkv"] for p in range(3) for c in range(NC))
            window = lambda ref: _cat([ref[:, HALO + r - DIL * w:HALO + r - DIL * w + 8, :] for w in range(W)], 1)
            qk = (_cat([after(q_s[:, r:r + 8, :], tok)] * W, 1) * window(k_s)).reshape(NC * W * 8, 128)
            logits = functools.reduce(jnp.add, [qk[c * W * 8:(c + 1) * W * 8] for c in range(NC)])
            if t in cfg["one_hop"]:
                slabs = [logits[8 * w:8 * w + 8] for w in range(W)]
                rolled = [[pltpu.roll(p, shift, 1) for shift in (32, 64, 96)] for p in slabs]
                yield
                a, b, c = [_cat(list(v), 0) for v in zip(*rolled)]
                logits = (logits + a) + (b + c)
            else:
                for shift in (64, 32):
                    rolled = pltpu.roll(logits, shift, 1)
                    yield
                    logits = logits + rolled
            if r < DIL * (W - 1):
                row = lax.broadcasted_iota(i32, logits.shape, 0)
                logits = jnp.where(r + (row & 7) >= DIL * (row >> 3), logits, -1e9 * LOG2E)
            e = jnp.exp2(logits - _cat([_fold(jnp.maximum, logits, 0)] * W, 0))
            norm = pl.reciprocal(_fold(jnp.add, e, 0), full_range=False)
            out = _fold(jnp.add, e * window(v_s), 1) * norm
            out = out.reshape(NC * 8, 128)
            out = [out[8 * c:8 * c + 8] for c in range(NC)]
            pending.append(_cat(out, 1))
            if len(pending) * 8 < G:
                return out
            group = _cat(pending, 0)
            pending.clear()
            return write_group(a_s, r + 8 - G, group)
        return [functools.partial(task, r) for r in range(t * TM, (t + 1) * TM, 8)]

    def products(key, r, rows, cols, tok, gated):
        m = [p[r:r + rows, cols] for p in vals[key]]
        return [after(v, tok) if i in gated else v for i, v in enumerate(m)]

    def second_norm(t):
        def task(j, tok):
            r = t * TM + G * j
            m = products(("proj", t), 16 * j, 16, slice(None), tok, (1, 2, 3))
            attended = _cat([_cat(_top(m), 1), _cat(_bottom(m), 1)], 0)
            vals["x1", r] = x1 = x_v[r:r + G, :].astype(f32) + vals["ga"] * attended
            y = yield from _layer_norm(x1)
            return write_group(y_s, r, (yield from _layer_norm(y * vals["cb"] + vals["sb"], GELU_A)))
        return [functools.partial(task, j) for j in range(NG)]

    def gelu(t, n0, width):
        pending = []

        def task(j, n, r, tok):
            m = products(("up", t, n0), 16 * j + r, 8, slice(n, n + 128), tok, (0, 2, 3))
            u = _cat(_top(m) + _bottom(m), 0)
            g = u + u * jnp.tanh(u * (GELU_K + u * u))
            pending.append([g[i:i + 8] for i in range(0, 32, 8)])
            if r == 0:
                return pending[0]
            quad = [_cat(p, 0) for p in zip(*pending)]
            pending.clear()
            return write_lhs(g_s, t * TM + G * j, n0 + n, quad)
        return [functools.partial(task, j, n, r)
                for j in range(NG) for n in range(0, width, 128) for r in (0, 8)]

    def out_copy(t, n=None):
        rows, cols = slice(t * TM, (t + 1) * TM), slice(0, D) if n is None else slice(n, n + 128)
        return pltpu.make_async_copy(o_v.at[rows, cols], o_hbm.at[0, rows, cols], out_sems.at[t + (n or 0) // 128])

    def finish(t):
        def task(r, tok):
            o = r % G
            half, gated = (_top, (2, 3)) if o < 16 else (_bottom, (1,))
            res = _cat(half(products(("down", t), (r % TM - o) // 2 + o % 16, 8, slice(None), tok, gated)), 1)
            out = vals["x1", r - o][o:o + 8] + vals["gb"] * res
            o_v[r:r + 8, :] = out.astype(bf16)
            if (r + 8) % TM == 0:
                out_copy(t).start()
            return [out[:, n:n + 128] for n in (0, D - 128)]
        return [functools.partial(task, r) for r in range(t * TM, (t + 1) * TM, 8)]

    def finish_columns(t, c, side):
        def task(j, tok):
            r, n = t * TM + G * j, c * 128 + HD * side
            m = [vals["down", t, i, c][16 * j:16 * j + 16] for i in range(7 - side)]
            if side:
                res = _cat([m[2] + m[4], ((m[0] - m[1]) + m[2]) + m[5]], 0)
            else:
                res = _cat([((m[0] + m[3]) - m[4]) + m[6], m[1] + m[3]], 0)
            out = vals["x1", r][:, n:n + 128] + vals["gb"][:, n:n + 128] * res
            o_v[r:r + G, n:n + 128] = out.astype(bf16)
            if j == NG - 1:
                out_copy(t, n).start()
        return [functools.partial(task, j) for j in range(NG)]

    stream, span, due = [], {}, []

    def clock():
        return stream[-1][0] + stream[-1][1] if stream else 0.0

    def strassen(key, left, t, right, n, width, bias=None):
        t0, cycles = clock(), HM * width / 256
        vals[key] = [None] * 7

        def store(i, m):
            if bias and i in (2, 3):
                col = n + (HF if i == 2 else 0)
                m = m + vals[bias][:, col:col + width]
            vals[key][i] = m
        for i in range(7):
            row = i * Q + t * TM // 4
            operand = (right, i * HD // 2, (i + 1) * HD // 2, n, n + width)
            if key[0] == "qkv" and i in (1, 4):
                k = HD * (i == 4)
                operand = (wp_s, k // 2, (k + HD) // 2, 2 * n + k, 2 * n + k + HD)
            stream.append((clock(), cycles, (left, row, row + TM // 4, 0, HD), operand, functools.partial(store, i)))
        span[key] = (t0, clock() - cycles, clock())

    def qkv_direct(t, part, k):
        t0 = clock()

        def store(n, m):
            if k == 0:
                vals["half", t, n] = m
                due.append((t0 + TM * (1 + n // HD % 2), [m[0:8, 0:128], m[0:8, 128:]]))
                return
            m = vals["half", t, n] + m
            for c in range(2):
                put_qkv(part, n % D // 128 + c, t * TM, m[:, c * 128:(c + 1) * 128])
        for n in (part * D, part * D + HD):
            stream.append((clock(), TM, (h0_s, t * HM, (t + 1) * HM, k, k + HD),
                           (wp_s, k // 2, (k + HD) // 2, n, n + HD), functools.partial(store, n)))
        span["direct", t, part, k] = (t0, clock() - TM, clock())

    def proj(t):
        strassen(("proj", t), a_s, t, tq_s, 3 * HD, HD)

    def up(t):
        for i, width in enumerate(UP_COLS):
            strassen(("up", t, sum(UP_COLS[:i])), y_s, t, t1_s, sum(UP_COLS[:i]), width, "b1")

    def down(t):
        t0 = clock()
        vals["down", t] = [None] * 7

        def store(i, c, k0, m):
            if k0:
                m = vals["down", t, i, c] + m
            elif i in (2, 3):
                n = c * 128 + (HD if i == 2 else 0)
                m = m + vals["b2"][:, n:n + 128]
            vals["down", t, i, c] = m
            if k0 and c:
                vals["down", t][i] = _cat([vals["down", t, i, 0], m], 1)
        order = [(i, c) for i in range(7) for c in range(2)]
        if t == NT - 1:
            order.sort(key=lambda ic: ic[1])
        for i, c in order:
            for k0, k1 in ((0, 512), (512, HF)):
                row = i * Q + t * TM // 4
                stream.append((clock(), HM * (k1 - k0) / 512, (g_s, row, row + TM // 4, k0, k1),
                               (t2_s, (i * HF + k0) // 2, (i * HF + k1) // 2, c * 128, (c + 1) * 128),
                               functools.partial(store, i, c, k0)))
            span["down", t, i, c] = span["down", t] = (t0, clock() - stream[-1][1], clock())

    for k in (0, HD):
        for part in range(3):
            for t in range(2):
                qkv_direct(t, part, k)
    for t in range(2, NT):
        for part in range(3):
            strassen(("qkv", t, part), h_s, t, tq_s, part * HD, HD)
        if t in cfg["proj_after"]:
            proj(cfg["proj_after"].index(t))
    up(0)
    for t in range(NT):
        if t + 2 < NT:
            proj(t + 2)
        if t + 1 < NT:
            up(t + 1)
        down(t)

    queue = []

    def pace(tasks, t0, t1, lag=None, at=0.5):
        for i, task in enumerate(tasks):
            when = t0 + (t1 - t0) * (i + at) / len(tasks)
            queue.append((when, len(queue), task, lag and lag + cfg["slack"]))

    def once(when, task, *args):
        pace([functools.partial(task, *args)], when, when)

    begin, final, end = [lambda *key, i=i: span[key][i] for i in range(3)]
    period, prep, early = 56 * HM, cfg["due_prep"], cfg["end_prep"]
    once(0, normalize, 1)
    once(0, modulate, 1, 0)
    once(begin("direct", 0, 1, 0) - cfg["lead_w"], interleave_heads, 0, D)
    once(begin("direct", 0, 2, 0) - cfg["lead_w"] - cfg["lead_w_more"], interleave_heads, 0, 2 * D)
    once(begin("direct", 0, 0, HD) - cfg["lead_mod"], shift_and_scale, HD)
    for t in range(2):
        once(begin("direct", 0, 0, HD) - cfg["lead_mod"], modulate, t, HD)
    once(begin("direct", 0, 0, HD) - cfg["lead_w_second"], interleave_heads, HD, 0)
    for part in (1, 2):
        once(begin("direct", 0, part, HD) - cfg["lead_w"] - cfg["lead_w_more"], interleave_heads, HD, part * D)
    pace(prepare_qkv(0), begin("direct", 1, 0, HD), begin("qkv", 2, 0) - early, prep)
    pace(prepare_qkv(1) + prepare_qkv(2), begin("qkv", 2, 0) - early, begin("qkv", 2, 2) - early - cfg["qkv_to"], prep)
    pace([column_of_c] + prepare_wo() + modulation(2, "ga", lambda v: v * (1.0 / QK_A))
         + modulation(3, "sb", lambda v: v) + modulation(4, "cb", lambda v: 1.0 + v),
         begin("qkv", 2, 2) - early - cfg["qkv_to"], begin("proj", 0) - early, prep)
    pace([biases] + prepare_w1(), begin("proj", 0) - early, begin("up", 0, HF - UP_COLS[-1]) - early, prep + cfg["due_w1"])
    pace(prepare_w2() + modulation(5, "gb", lambda v: v * (0.5 / GELU_A)),
         begin("up", 0, HF - UP_COLS[-1]) - cfg["w2_from"] * 7 * HM, begin("down", 0) - early + cfg["w2_to"], prep + cfg["due_w2"])
    free = dict(ln1=begin("direct", 0, 1, HD), attn=begin("qkv", 2, 0), ln23=0.0, gelu=0.0)
    for t in range(NT):
        if t >= 2:
            for part in range(3):
                pace(split_qkv(t, part), final("qkv", t, part), end("qkv", t, part), at=1.0)
            t0, free["ln1"] = free["ln1"], begin("qkv", t, 0) - cfg["end_ln1"]
            pace(first_norm(t), t0, free["ln1"], cfg["due_ln1"])
        t0 = free["attn"]
        free["attn"] = t0 + min((begin("proj", u) - cfg["end_attn"] - t0) / (u - t + 1) for u in range(t, NT))
        pace(attention(t), t0, free["attn"], cfg["due_attn"], cfg["at_attn"])
        t1 = begin("up", t, 0) - cfg["end_ln23"]
        t0 = max(end("proj", t), t1 - cfg["len_ln23"] * period, free["ln23"])
        free["ln23"] = max(t0, t1)
        pace(second_norm(t), t0, max(t1, end("proj", t)), cfg["due_ln23"], cfg["at_ln23"])
        t0 = max(end("up", t, 0), free["gelu"])
        free["gelu"] = t1 = min(begin("down", t) - cfg["end_gelu"], t0 + period)
        for i, width in enumerate(UP_COLS):
            n = sum(UP_COLS[:i])
            lo = max(end("up", t, n), t0 + (t1 - t0) * n / HF)
            pace(gelu(t, n, width), lo, max(lo, t0 + (t1 - t0) * (n + width) / HF), cfg["due_gelu"])
        if t < NT - 1:
            pace(finish(t), end("down", t), end("down", t) + cfg["len_out"] * HM, cfg["due_out"])
        else:
            for c in range(2):
                for side in (1, 0):
                    key = ("down", t, 6 - side, c)
                    pace(finish_columns(t, c, side), final(*key), end(*key), at=1.0)
    heapq.heapify(queue)

    def run_next(tick, tick_end):
        when, seq, task, lag = heapq.heappop(queue)
        if callable(task):
            r = 8 * int(min(max(when - tick_end + tick.shape[0], 0.0), tick.shape[0] - 1) / 8)
            task = task(tick[r:r + 8])
        if hasattr(task, "send"):
            try:
                next(task)
                heapq.heappush(queue, (when + cfg["step"], seq, task, lag - cfg["step"]))
                return
            except StopIteration as stop:
                task = stop.value
        if lag and task:
            due.append((when + lag, task))

    normalize(0, start)
    shift_and_scale(0, vals["xn", 0][TM - 8:, D - 128:])
    interleave_heads(0, 0, _fold(jnp.maximum, modulate(0, 0, None)[:, 0:128], 0))

    issued, tick, tick_end = 0.0, None, 0.0
    for t0, cycles, left, right, store in stream:
        while True:
            try:
                a, b = read(*left), read(*right)
                break
            except _NotReady:
                run_next(tick, tick_end)
        ties = {}
        for when, toks in due:
            if when < t0 + cycles:
                ties.setdefault(8 * int(max(when - t0, 0.0) / cycles * a.shape[0] / 8), []).extend(toks)
        due[:] = [d for d in due if d[0] >= t0 + cycles]
        for r, toks in ties.items():
            a = after_rows(a, r, toks)
        res = jnp.dot(_unpack(a), _unpack(b), preferred_element_type=f32)
        store(res)
        m = res.shape[0]
        for n in range(0, res.shape[1], 128):
            issued += m * (a.shape[1] // 128) / 4
            round_end = math.ceil(issued / m - 1e-6) * m
            if round_end > tick_end:
                tick, tick_end = res[:, n:n + 128], round_end
                while queue and queue[0][0] <= min(tick_end, t0 + cycles) + 1e-6:
                    run_next(tick, tick_end)
    while queue:
        run_next(tick, tick_end)
    for t in range(NT - 1):
        out_copy(t).wait()
    for n in (HD, 0, HD + 128, 128):
        out_copy(NT - 1, n).wait()


@jax.jit
def pallas_adaLN_cond__sliding_local_dilated__mixer_channel_mlp__prompt_kernel(
        A_x, A_wqkv, A_wo, B_x, B_w1, B_b1, B_w2, B_b2, c, w_mod):
    del B_x
    inputs = (A_x, A_wqkv, A_wo, B_w1, B_b1, B_w2, B_b2, c, w_mod)
    return pl.pallas_call(
        _kernel,
        out_shape=jax.ShapeDtypeStruct(A_x.shape, A_x.dtype),
        in_specs=[pl.BlockSpec(memory_space=pl.ANY)] * len(inputs),
        out_specs=pl.BlockSpec(memory_space=pl.ANY),
        scratch_shapes=[
            pltpu.VMEM((S, D), bf16),
            pltpu.VMEM((D, 3 * D), bf16),
            pltpu.VMEM((D, D), bf16),
            pltpu.VMEM((D, F), bf16),
            pltpu.VMEM((F, D), bf16),
            pltpu.VMEM((D, 6 * D), bf16),
            pltpu.VMEM((F,), bf16),
            pltpu.VMEM((D,), bf16),
            pltpu.VMEM((1, D), bf16),
            pltpu.VMEM((S, D), bf16),
            pltpu.VMEM((D // 2, 3 * D), i32),
            pltpu.VMEM((NC, D, 128), f32),
            pltpu.VMEM((7 * HD // 2, 4 * HD), i32),
            pltpu.VMEM((7 * HD // 2, HF), i32),
            pltpu.VMEM((7 * HF // 2, HD), i32),
            pltpu.VMEM((D, 128), f32),
            pltpu.VMEM((TM, D), i32),
            pltpu.VMEM((7 * Q, HD), i32),
            pltpu.VMEM((7 * Q, HD), i32),
            pltpu.VMEM((7 * Q, HD), i32),
            pltpu.VMEM((7 * Q, HF), i32),
            pltpu.VMEM((NC, S, 128), f32),
            pltpu.VMEM((NC, HALO + S, 128), f32),
            pltpu.VMEM((NC, HALO + S, 128), f32),
            pltpu.SemaphoreType.DMA((24,)),
            pltpu.SemaphoreType.DMA((NT + 3,)),
        ],
        compiler_params=pltpu.CompilerParams(
            vmem_limit_bytes=110 * 1024 * 1024,
            flags={"XLA_TPU_RESCHEDULE_DMA_DONES": True},
            disable_semaphore_checks=True,
            disable_bounds_checks=True,
        ),
    )(*inputs)
```
